```python
import os as _os
_os.environ.setdefault("JAX_PLATFORMS", "cpu")
import jax
import jax.numpy as jnp

def _softmax(x, axis=-1):
    return jax.nn.softmax(x, axis=axis)
def _gelu(x):
    return jax.nn.gelu(x, approximate=True)
def _silu(x):
    return jax.nn.silu(x)
def _sigmoid(x):
    return jax.nn.sigmoid(x)
def _layernorm(x, axis=-1, eps=1e-5):
    m = jnp.mean(x, axis=axis, keepdims=True)
    v = jnp.var(x, axis=axis, keepdims=True)
    return (x - m) / jnp.sqrt(v + eps)
def _scatter_add(tgt, idx, src, axis=0):
    return tgt.at[idx].add(src)
def _segment_sum(src, seg, n):
    return jax.ops.segment_sum(src, seg, n)
class _Rng:
    def __init__(self, key):
        self._k = key
    def _next(self):
        self._k, sub = jax.random.split(self._k)
        return sub
    def normal(self, shape):
        return jax.random.normal(self._next(), shape, dtype=jnp.bfloat16)
    def randint(self, lo, hi, shape):
        return jax.random.randint(self._next(), shape, lo, hi, dtype=jnp.int32)
    def uniform(self, shape, lo=0.0, hi=1.0):
        return jax.random.uniform(self._next(), shape, jnp.bfloat16, lo, hi)
    def permutation(self, n):
        return jax.random.permutation(self._next(), n)


kernel_name = 'gated_mix__sliding_local_dilated__moe_arch_mod__prompt'

def setup_inputs():
    _rng = _Rng(jax.random.key(int.from_bytes(__import__("os").urandom(4), "little")))
    _w = (lambda a: (lambda t: t.astype(jnp.bfloat16) if jnp.issubdtype(t.dtype, jnp.floating) else t)(jnp.asarray(a)))
    def _A_setup():
        B, S, D = 1, 2048, 640
        return {
            "x": _w((lambda *s: _rng.normal(s) * 0.05)(B, S, D)),
            "wqkv": _w((lambda *s: _rng.normal(s) * 0.8)(D, 3 * D)),
            "wo": _w((lambda *s: _rng.normal(s) * 0.05)(D, D)),
        }
    _A_in = _A_setup()

    def _B_setup():
        B, S, D, F, C = 1, 2048, 640, 1728, 1
        return {
            "x": _w((lambda *s: _rng.normal(s) * 0.05)(B, S, D)),
            "w_r": _w((lambda *s: _rng.normal(s) * 1.6)(D)),
            "w_gate": _w((lambda *s: _rng.normal(s) * 0.4)(D, F)),
            "w_up": _w((lambda *s: _rng.normal(s) * 0.4)(D, F)),
            "w_down": _w((lambda *s: _rng.normal(s) * 0.4)(F, D)),
        }
    _B_in = _B_setup()

    return {
        "A_x": _A_in["x"],
        "A_wqkv": _A_in["wqkv"],
        "A_wo": _A_in["wo"],
        "B_x": _B_in["x"],
        "B_w_r": _B_in["w_r"],
        "B_w_gate": _B_in["w_gate"],
        "B_w_up": _B_in["w_up"],
        "B_w_down": _B_in["w_down"],
        "gate_w": _w((lambda *s: _rng.normal(s) * 0.05)(640) * 16.0),
    }

def reference(A_x, A_wqkv, A_wo, B_x, B_w_r, B_w_gate, B_w_up, B_w_down, gate_w):
    def _A_ref(x, wqkv, wo):
        B, S, D = x.shape
        H = 32; Dh = D // H
        W, dil = 8, 2
        qkv = (lambda x, *d: x.transpose(*d))((x @ wqkv).reshape(B, S, 3, H, Dh), 2, 0, 3, 1, 4)
        q, k, v = qkv[0], qkv[1], qkv[2]
        scale = Dh ** -0.5
        pos = jnp.arange(S)
        off = jnp.arange(W) * dil
        idx = pos[:, None] - off[None, :]
        mask = idx >= 0
        idx_c = jnp.where(mask, idx, 0).reshape(-1)
        kg = k[:, :, idx_c, :].reshape(B, H, S, W, Dh)
        vg = v[:, :, idx_c, :].reshape(B, H, S, W, Dh)
        logits = jnp.einsum("bhsd,bhswd->bhsw", q, kg) * scale
        logits = jnp.where(mask[None, None, :, :], logits, -1e9)
        attn = _softmax(logits, axis=-1)
        o = jnp.einsum("bhsw,bhswd->bhsd", attn, vg)
        return (lambda x, *d: x.transpose(*d))(o, 0, 2, 1, 3).reshape(B, S, D) @ wo

    def _B_ref(x, w_r, w_gate, w_up, w_down):
        B, S, D = x.shape
        C = 1
        r = x @ w_r
        idx = jnp.argsort(-r, axis=-1)[:, :C]
        idx_e = jnp.repeat(idx.reshape(B, C, 1), D, axis=2)
        x_sel = jnp.take_along_axis(x, idx_e, axis=1)
        g = _silu(x_sel @ w_gate)
        u = x_sel @ w_up
        y = (g * u) @ w_down
        r_sel = _sigmoid(jnp.take_along_axis(r, idx, axis=1))
        y = y * r_sel.reshape(B, C, 1)
        b_off = (jnp.arange(B) * S).reshape(B, 1)
        flat_idx = (idx + b_off).reshape(B * C)
        zero = (x * 0.0).reshape(B * S, D)
        upd = _scatter_add(zero, flat_idx, y.reshape(B * C, D), axis=0)
        return x + upd.reshape(B, S, D)

    x = A_x
    g = _sigmoid((x * gate_w).sum(-1, keepdims=True))
    a = _A_ref(x, A_wqkv, A_wo)
    b = _B_ref(x, B_w_r, B_w_gate, B_w_up, B_w_down)
    return g * a + (1 - g) * b
```

```python
import functools
import numpy as np
import jax
import jax.numpy as jnp
from jax import lax
import jax.experimental.pallas as pl
import jax.experimental.pallas.tpu as pltpu

S, D, H, DH, NW, DIL, F = 2048, 640, 32, 20, 8, 2, 1728
NT = D // 128
HALO = 16
M = 256
R = 32
NG = 3
PM = 128
ORD = 'qqpqpqq'
NB = S // M
UNROLL = 0
LAG = 1
ROT3 = 1
QSCALE = float(DH ** -0.5 * np.log2(np.e))
NEG = float(-1e9 * np.log2(np.e))
f32, bf16, u32, i32 = jnp.float32, jnp.bfloat16, jnp.uint32, jnp.int32
NT_DIMS = (((1,), (1,)), ((), ()))


def _permute_rows(words, tmp, dst, row0):
    for c in range(NT):
        tmp[c] = words[:, c * 128:(c + 1) * 128]
    for c in range(NT):
        for dp in range(DH // 2):
            for hh in range(2):
                ev = tmp[c, pl.ds(hh * 160 + dp, 8, stride=20), :]
                od = tmp[c, pl.ds(hh * 160 + 10 + dp, 8, stride=20), :]
                lo = (ev & u32(0xFFFF)) | (od << 16)
                hi = (ev >> 16) | (od & u32(0xFFFF0000))
                r = row0 + dp * 32 + hh * 8
                dst[r:r + 8, c * 128:(c + 1) * 128] = lo
                dst[r + 16:r + 24, c * 128:(c + 1) * 128] = hi


def _interleave(*lists):
    ev = []
    for n, tasks in enumerate(lists):
        total = sum(w for w, _ in tasks) or 1
        acc = 0
        for k, (w, t) in enumerate(tasks):
            ev.append((acc / total, n, k, t))
            acc += w
    for e in sorted(ev, key=lambda e: e[:3]):
        e[3]()


def _kernel(x_hbm, wqkv_hbm, wo_hbm, wr_ref, wg_hbm, wu_hbm, wd_hbm, gw_ref, out_hbm,
            x_v, wqkv_v, wo_v, wg_v, wu_v, wd_v, tmp, wt, wop,
            buf, lbuf, obuf, xp, gbuf, best, out_v, isem, osem):
    def x_copy(r0, n, k):
        return pltpu.make_async_copy(x_hbm.at[0, pl.ds(r0, n)], x_v.at[pl.ds(r0, n)], isem.at[k])
    cp_x = [x_copy(0, M, 0), x_copy(M, M, 9), x_copy(2 * M, M, 4), x_copy(3 * M, S - 3 * M, 10)]
    cp_w = [pltpu.make_async_copy(wqkv_hbm.at[:, pl.ds(j * D, D)], wqkv_v.at[j], isem.at[1 + j]) for j in range(3)]
    cp_wo = pltpu.make_async_copy(wo_hbm, wo_v, isem.at[5])
    cp_f = [pltpu.make_async_copy(a, b, isem.at[6 + j]) for j, (a, b) in
            enumerate(((wg_hbm, wg_v), (wu_hbm, wu_v), (wd_hbm, wd_v)))]
    cp_x[0].start()
    cp_w[0].start()

    gw = gw_ref[...].astype(f32).reshape(1, D)
    wr = wr_ref[...].astype(f32).reshape(1, D)

    def stage(i):
        tasks = []
        for p0 in range(0, M, 64):
            def task(p0=p0):
                r0 = pl.multiple_of(i32(i * M + p0), 64)
                xb = x_v[pl.ds(r0, 64), :]
                xp[pl.ds(pl.multiple_of(r0 // 2, 32), 32), :] = pltpu.bitcast(xb, u32)
                xf = xb.astype(f32)
                g = jax.nn.sigmoid(jnp.sum(xf * gw, axis=-1, keepdims=True))
                gbuf[pl.ds(r0, 64), :] = jnp.broadcast_to(g, (64, 128))
                r = jnp.sum(xf * wr, axis=-1, keepdims=True).astype(bf16).astype(f32)
                bv, bi = best[0], best[1]
                for a in range(0, 64, 8):
                    ra = jnp.broadcast_to(r[a:a + 8], (8, 128))
                    up = ra > bv
                    bv = jnp.where(up, ra, bv)
                    bi = jnp.where(up, (r0 + a).astype(f32), bi)
                best[0] = bv
                best[1] = bi
            tasks.append((1, task))
        return tasks

    def qkv(i, NG=NG):
        sl = i % 2
        tasks = []
        for t0 in range(0, 3 * NT, NG):
            def task(t0=t0):
                xb = pltpu.bitcast(xp[pl.ds(pl.multiple_of(i * (M // 2), M // 2), M // 2), :], bf16)
                w = pltpu.bitcast(wt[t0 * 64:(t0 + NG) * 64, :], bf16)
                y = lax.dot_general(xb, w, NT_DIMS, preferred_element_type=f32)
                for t in range(NG):
                    yc = y[:, t * 128:(t + 1) * 128]
                    buf[sl, t0 + t, HALO:HALO + M, :] = yc * QSCALE if t0 + t < NT else yc
            tasks.append((NG * M, task))
        return tasks

    def prep_w(j):
        _permute_rows(pltpu.bitcast(wqkv_v[j].T, u32), tmp, wt, j * (D // 2))

    def halo(i):
        for c in range(NT, 3 * NT):
            buf[(i + 1) % 2, c, 0:HALO, :] = buf[i % 2, c, M:M + HALO, :]

    def attn(i):
        sl = i % 2
        p1, p3 = [], []
        for r0 in range(0, M, R):
            def logits(r0=r0):
                q = [buf[sl, c, HALO + r0:HALO + r0 + R, :] for c in range(NT)]
                for w in range(NW):
                    o = HALO + r0 - DIL * w
                    l = q[0] * buf[sl, NT, o:o + R, :]
                    for c in range(1, NT):
                        l = l + q[c] * buf[sl, NT + c, o:o + R, :]
                    if ROT3:
                        l = (l + pltpu.roll(l, 64, 1)) + (pltpu.roll(l, 32, 1) + pltpu.roll(l, 96, 1))
                    else:
                        l = l + pltpu.roll(l, 64, 1)
                        l = l + pltpu.roll(l, 32, 1)
                    if r0 < DIL * w:
                        pos = lax.broadcasted_iota(i32, (R, 128), 0) + (i * M + r0)
                        l = jnp.where(pos >= DIL * w, l, NEG)
                    lbuf[w, r0:r0 + R, :] = l

            def mix(r0=r0):
                ls = [lbuf[w, r0:r0 + R, :] for w in range(NW)]
                m = functools.reduce(jnp.maximum, ls)
                ps = [jnp.exp2(l - m) for l in ls]
                inv = 1.0 / functools.reduce(lambda a, b: a + b, ps)
                for c in range(NT):
                    acc = None
                    for w in range(NW):
                        o = HALO + r0 - DIL * w
                        t = ps[w] * buf[sl, 2 * NT + c, o:o + R, :]
                        acc = t if acc is None else acc + t
                    obuf[sl, r0 // 2:(r0 + R) // 2, c * 128:(c + 1) * 128] = pltpu.bitcast((acc * inv).astype(bf16), u32)
            p1.append((1, logits))
            p3.append((1, mix))
        n = len(p1)
        tasks = p1[:LAG]
        for j in range(n):
            if j + LAG < n:
                tasks.append(p1[j + LAG])
            tasks.append(p3[j])
        return tasks

    def proj(i):
        sl = i % 2
        tasks = []
        for p0 in range(0, M, PM):
            def task(p0=p0):
                r0 = pl.multiple_of(i * M + p0, PM)
                a = jnp.dot(pltpu.bitcast(obuf[sl, p0 // 2:(p0 + PM) // 2, :], bf16), pltpu.bitcast(wop[...], bf16),
                            preferred_element_type=f32)
                xf = pltpu.bitcast(xp[pl.ds(pl.multiple_of(r0 // 2, PM // 2), PM // 2), :], bf16).astype(f32)
                g = gbuf[pl.ds(r0, PM), :]
                g = jnp.concatenate([g] * NT, axis=1)
                out_v[pl.ds(r0, PM), :] = (xf + g * (a - xf)).astype(bf16)
            tasks.append((NT * PM, task))
        return tasks

    def out_copy(i):
        r0 = pl.multiple_of(i * M, M)
        return pltpu.make_async_copy(out_v.at[pl.ds(r0, M)], out_hbm.at[0, pl.ds(r0, M)], osem.at[i])

    def mxu_order(q, p):
        q, p = list(q), list(p)
        out = [(q if ch == "q" else p).pop(0) for ch in ORD if (q if ch == "q" else p)]
        return out + q + p

    best[0] = jnp.full((8, 128), -jnp.inf, f32)
    best[1] = jnp.zeros((8, 128), f32)
    q0 = qkv(0, NT)
    cp_x[0].wait()
    cp_w[1].start()
    _interleave(stage(0))
    cp_w[0].wait()
    cp_w[2].start()
    prep_w(0)
    cp_w[1].wait()
    cp_x[1].start()
    cp_x[2].start()
    q0[0][1]()
    prep_w(1)
    cp_w[2].wait()
    cp_wo.start()
    cp_x[3].start()
    q0[1][1]()
    prep_w(2)
    cp_x[1].wait()
    _interleave(q0[2:], stage(1))
    for c in range(NT, 3 * NT):
        buf[0, c, 0:HALO, :] = jnp.broadcast_to(buf[0, c, HALO:HALO + 1, :], (HALO, 128))
    cp_x[2].wait()
    cp_wo.wait()
    halo(0)
    _interleave(qkv(1), attn(0) + stage(2))
    _permute_rows(pltpu.bitcast(wo_v[...], u32), tmp, wop, 0)
    cp_x[3].wait()
    for c in cp_f:
        c.start()

    def step(i, carry):
        @pl.when(i >= 2)
        def _():
            out_copy(i - 2).start()
        halo(i)
        _interleave(mxu_order(qkv(i + 1), proj(i - 1)), attn(i) + stage(jnp.minimum(i + 2, NB - 1)))
        return carry
    if UNROLL:
        for i in range(1, NB - 1):
            if i >= 2:
                out_copy(i - 2).start()
            halo(i)
            _interleave(mxu_order(qkv(i + 1), proj(i - 1)), attn(i) + (stage(i + 2) if i + 2 < NB else []))
    else:
        lax.fori_loop(1, NB - 1, step, 0)
    out_copy(NB - 3).start()

    bv, bi = best[0], best[1]
    rmax = jnp.max(bv, axis=0, keepdims=True)
    pos = bi + lax.broadcasted_iota(i32, (8, 128), 0).astype(f32)
    idx = jnp.min(jnp.where(bv == rmax, pos, float(S - 1))).astype(i32)
    t0 = pl.multiple_of((idx // 16) * 16, 16)
    sel = lax.broadcasted_iota(i32, (16, D), 0) == (idx - t0)
    for c in cp_f:
        c.wait()
    res = []

    def ffn():
        xt = x_v[pl.ds(t0, 16), :].astype(f32)
        xs = jnp.sum(jnp.where(sel, xt, 0.0), axis=0, keepdims=True)
        xs16 = jnp.broadcast_to(xs, (16, D)).astype(bf16)
        gg = lax.dot_general(xs16, wg_v[...], NT_DIMS, preferred_element_type=f32)
        uu = lax.dot_general(xs16, wu_v[...], NT_DIMS, preferred_element_type=f32)
        hh = (gg * jax.nn.sigmoid(gg) * uu).astype(bf16)
        y = jnp.dot(hh, wd_v[...], preferred_element_type=f32)
        gs = jax.nn.sigmoid(jnp.sum(xs * gw, axis=-1, keepdims=True))
        res.append(y * jax.nn.sigmoid(rmax[:, 0:1]) * (1.0 - gs))

    _interleave(proj(NB - 2) + [(1, ffn)], attn(NB - 1))
    _interleave(proj(NB - 1))
    for i in range(NB - 2):
        out_copy(i).wait()
    ot = out_v[pl.ds(t0, 16), :].astype(f32)
    out_v[pl.ds(t0, 16), :] = jnp.where(sel, ot + res[0], ot).astype(bf16)
    out_copy(NB - 2).start()
    out_copy(NB - 1).start()

    @pl.when(idx < (NB - 2) * M)
    def _():
        cp = pltpu.make_async_copy(out_v.at[pl.ds(t0, 16)], out_hbm.at[0, pl.ds(t0, 16)], osem.at[0])
        cp.start()
        cp.wait()
    out_copy(NB - 2).wait()
    out_copy(NB - 1).wait()


@jax.jit
def pallas_gated_mix__sliding_local_dilated__moe_arch_mod__prompt_kernel(A_x, A_wqkv, A_wo, B_x, B_w_r, B_w_gate, B_w_up, B_w_down, gate_w):
    del B_x
    anyspec = pl.BlockSpec(memory_space=pl.ANY)
    vspec = pl.BlockSpec(memory_space=pltpu.VMEM)
    return pl.pallas_call(
        _kernel,
        out_shape=jax.ShapeDtypeStruct((1, S, D), bf16),
        in_specs=[anyspec, anyspec, anyspec, vspec, anyspec, anyspec, anyspec, vspec],
        out_specs=anyspec,
        scratch_shapes=[
            pltpu.VMEM((S, D), bf16), pltpu.VMEM((3, D, D), bf16), pltpu.VMEM((D, D), bf16),
            pltpu.VMEM((F, D), bf16), pltpu.VMEM((F, D), bf16), pltpu.VMEM((F, D), bf16),
            pltpu.VMEM((NT, D // 2, 128), u32), pltpu.VMEM((3 * D // 2, D), u32), pltpu.VMEM((D // 2, D), u32),
            pltpu.VMEM((2, 3 * NT, M + HALO, 128), f32), pltpu.VMEM((NW, M, 128), f32), pltpu.VMEM((2, M // 2, D), u32),
            pltpu.VMEM((S // 2, D), u32), pltpu.VMEM((S, 128), f32), pltpu.VMEM((2, 8, 128), f32),
            pltpu.VMEM((S, D), bf16),
            pltpu.SemaphoreType.DMA((11,)), pltpu.SemaphoreType.DMA((NB,)),
        ],
        compiler_params=pltpu.CompilerParams(vmem_limit_bytes=100 << 20),
        name="gmix",
    )(A_x, A_wqkv, A_wo, B_w_r, B_w_gate.T, B_w_up.T, B_w_down, gate_w)
```

```python
import functools

import numpy as np
import jax
import jax.numpy as jnp
from jax import lax
import jax.experimental.pallas as pl
import jax.experimental.pallas.tpu as pltpu

S, D, DH, NW, DIL, F = 2048, 640, 20, 8, 2, 1728
NT = D // 128
HALO = 16
M = 256
NB = S // M
R = 32
SR = 64
PM = 128
NG = 3
LAG = 3
TAPS = (0, 4, 1, 5, 2, 6, 3, 7)
LOG2E = float(np.log2(np.e))
QSCALE = float(DH ** -0.5) * LOG2E
NEG = -1e9 * LOG2E
f32, bf16, u32, i32 = jnp.float32, jnp.bfloat16, jnp.uint32, jnp.int32
NT_DIMS = (((1,), (1,)), ((), ()))


def _permute_rows(words, tmp, dst, row0):
    for c in range(NT):
        tmp[c] = words[:, c * 128:(c + 1) * 128]
    for c in range(NT):
        for dp in range(DH // 2):
            for hh in range(2):
                ev = tmp[c, pl.ds(hh * 160 + dp, 8, stride=20), :]
                od = tmp[c, pl.ds(hh * 160 + 10 + dp, 8, stride=20), :]
                lo = (ev & u32(0xFFFF)) | (od << 16)
                hi = (ev >> 16) | (od & u32(0xFFFF0000))
                r = row0 + dp * 32 + hh * 8
                dst[r:r + 8, c * 128:(c + 1) * 128] = lo
                dst[r + 16:r + 24, c * 128:(c + 1) * 128] = hi


def _windows(load, base):
    cache = {}

    def win(c, w):
        key = (c, w % 4)
        if key not in cache:
            cache[key] = load(c, base - DIL * (w % 4) - 8, R + 8)
        off = 0 if w >= 4 else 8
        return cache[key][off:off + R]
    return win


def _interleave(*lists, span=1.0):
    ev = []
    for n, tasks in enumerate(lists):
        total = sum(w for w, _ in tasks) or 1
        acc = 0
        for k, (w, t) in enumerate(tasks):
            ev.append((acc / total * (span if n else 1.0), n, k, t))
            acc += w
    for e in sorted(ev, key=lambda e: e[:3]):
        e[3]()


def _kernel(x_hbm, wqkv_hbm, wo_hbm, wr_ref, wg_hbm, wu_hbm, wd_hbm, gw_ref, out_hbm,
            x_v, wqkv_v, wo_v, wg_v, wu_v, wd_v, tmp, wt, wop,
            buf, lbuf, obuf, xp, gbuf, best, out_v, isem, osem, lsem):
    def x_copy(r0, n, k):
        return pltpu.make_async_copy(x_hbm.at[0, pl.ds(r0, n)], x_v.at[pl.ds(r0, n)], isem.at[k])

    cp_x = [x_copy(0, M, 0), x_copy(M, M, 9), x_copy(2 * M, M, 4), x_copy(3 * M, S - 3 * M, 10)]
    cp_w = [pltpu.make_async_copy(wqkv_hbm.at[:, pl.ds(j * D, D)], wqkv_v.at[j], isem.at[1 + j])
            for j in range(3)]
    cp_wo = pltpu.make_async_copy(wo_hbm, wo_v, isem.at[5])
    cp_f = [pltpu.make_async_copy(a, b, isem.at[6 + j]) for j, (a, b) in
            enumerate(((wg_hbm, wg_v), (wu_hbm, wu_v), (wd_hbm, wd_v)))]
    cp_x[0].start()
    cp_w[0].start()

    gw = gw_ref[...].astype(f32).reshape(1, D)
    wr = wr_ref[...].astype(f32).reshape(1, D)

    def stage(i):
        tasks = []
        for p0 in range(0, M, SR):
            def task(p0=p0):
                r0 = pl.multiple_of(i32(i * M + p0), SR)
                xb = x_v[pl.ds(r0, SR), :]
                xp[pl.ds(pl.multiple_of(r0 // 2, SR // 2), SR // 2), :] = pltpu.bitcast(xb, u32)
                xf = xb.astype(f32)
                g = jax.nn.sigmoid(jnp.sum(xf * gw, axis=-1, keepdims=True))
                gbuf[pl.ds(r0, SR), :] = jnp.broadcast_to(g, (SR, 128))
                r = jnp.sum(xf * wr, axis=-1, keepdims=True).astype(bf16).astype(f32)
                bv, bi = best[0], best[1]
                for a in range(0, SR, 8):
                    ra = jnp.broadcast_to(r[a:a + 8], (8, 128))
                    up = ra > bv
                    bv = jnp.where(up, ra, bv)
                    bi = jnp.where(up, (r0 + a).astype(f32), bi)
                best[0] = bv
                best[1] = bi
            tasks.append((1, task))
        return tasks

    def qkv(i, ng=NG):
        sl = i % 2
        tasks = []
        for t0 in range(0, 3 * NT, ng):
            def task(t0=t0):
                xb = pltpu.bitcast(xp[pl.ds(pl.multiple_of(i * (M // 2), M // 2), M // 2), :], bf16)
                w = pltpu.bitcast(wt[t0 * 64:(t0 + ng) * 64, :], bf16)
                y = lax.dot_general(xb, w, NT_DIMS, preferred_element_type=f32)
                for t in range(ng):
                    yc = y[:, t * 128:(t + 1) * 128]
                    buf[sl, t0 + t, HALO:HALO + M, :] = yc * QSCALE if t0 + t < NT else yc
            tasks.append((ng * M, task))
        return tasks

    def prep_w(j):
        _permute_rows(pltpu.bitcast(wqkv_v[j].T, u32), tmp, wt, j * (D // 2))

    def halo(i, lo=NT, hi=3 * NT):
        for c in range(lo, hi):
            buf[(i + 1) % 2, c, 0:HALO, :] = buf[i % 2, c, M:M + HALO, :]

    def first_halo(lo, hi):
        for c in range(lo, hi):
            buf[0, c, 0:HALO, :] = jnp.broadcast_to(buf[0, c, HALO:HALO + 1, :], (HALO, 128))

    def attn(i, split=False):
        sl = i % 2
        p1, p3 = [], []
        for r0 in range(0, M, R):
            def logits(r0=r0):
                q = [buf[sl, c, HALO + r0:HALO + r0 + R, :] for c in range(NT)]
                win = _windows(lambda c, o, n: buf[sl, NT + c, o:o + n, :], HALO + r0)
                for w in TAPS:
                    l = functools.reduce(jnp.add, [q[c] * win(c, w) for c in range(NT)])
                    l = (l + pltpu.roll(l, 64, 1)) + (pltpu.roll(l, 32, 1) + pltpu.roll(l, 96, 1))
                    if r0 < DIL * w:
                        pos = lax.broadcasted_iota(i32, (R, 128), 0) + (i * M + r0)
                        l = jnp.where(pos >= DIL * w, l, NEG)
                    lbuf[w, r0:r0 + R, :] = l

            def mix(r0=r0):
                ls = [lbuf[w, r0:r0 + R, :] for w in range(NW)]
                m = functools.reduce(jnp.maximum, ls)
                ps = [jnp.exp2(l - m) for l in ls]
                win = _windows(lambda c, o, n: buf[sl, 2 * NT + c, o:o + n, :], HALO + r0)
                inv = 1.0 / functools.reduce(jnp.add, ps)
                for c in range(NT):
                    acc = functools.reduce(jnp.add, [ps[w] * win(c, w) for w in TAPS])
                    obuf[sl, r0 // 2:(r0 + R) // 2, c * 128:(c + 1) * 128] = pltpu.bitcast(
                        (acc * inv).astype(bf16), u32)
            p1.append((1, logits))
            p3.append((1, mix))
        if split:
            return p1, p3
        tasks = p1[:LAG]
        for j in range(len(p1)):
            if j + LAG < len(p1):
                tasks.append(p1[j + LAG])
            tasks.append(p3[j])
        return tasks

    def out_copy(i):
        r0 = pl.multiple_of(i * M, M)
        return pltpu.make_async_copy(out_v.at[pl.ds(r0, M)], out_hbm.at[0, pl.ds(r0, M)], osem.at[i])

    def last_copy(p0):
        r0 = (NB - 1) * M + p0
        return pltpu.make_async_copy(out_v.at[pl.ds(r0, PM)], out_hbm.at[0, pl.ds(r0, PM)],
                                     lsem.at[p0 // PM])

    def proj(i, patch=None):
        sl = i % 2
        tasks = []
        for p0 in range(0, M, PM):
            def task(p0=p0):
                r0 = pl.multiple_of(i * M + p0, PM)
                a = jnp.dot(pltpu.bitcast(obuf[sl, p0 // 2:(p0 + PM) // 2, :], bf16),
                            pltpu.bitcast(wop[...], bf16), preferred_element_type=f32)
                xf = pltpu.bitcast(xp[pl.ds(pl.multiple_of(r0 // 2, PM // 2), PM // 2), :], bf16).astype(f32)
                g = gbuf[pl.ds(r0, PM), :]
                g = jnp.concatenate([g] * NT, axis=1)
                o = xf + g * (a - xf)
                if patch is not None:
                    o = jnp.where(lax.broadcasted_iota(i32, (PM, D), 0) == patch[0] - r0,
                                  o + patch[1][0:1], o)
                out_v[pl.ds(r0, PM), :] = o.astype(bf16)
                if patch is not None:
                    last_copy(p0).start()
            tasks.append((NT * PM, task))
        return tasks

    best[0] = jnp.full((8, 128), -jnp.inf, f32)
    best[1] = jnp.zeros((8, 128), f32)
    q0, q1 = qkv(0, NT), qkv(1, NT)
    lg0, mx0 = attn(0, split=True)
    cp_x[0].wait()
    cp_x[1].start()
    _interleave(stage(0)[:2])
    cp_w[0].wait()
    cp_w[1].start()
    prep_w(0)
    _interleave(stage(0)[2:])
    cp_w[2].start()
    cp_x[1].wait()
    _interleave(q0[0:1], stage(1))
    cp_x[2].start()
    cp_wo.start()
    cp_w[1].wait()
    _interleave(q1[0:1])
    prep_w(1)
    cp_x[3].start()
    cp_w[2].wait()
    _interleave(q0[1:2])
    first_halo(NT, 2 * NT)
    halo(0, NT, 2 * NT)
    prep_w(2)
    _interleave(lg0 + q1[1:2] + q0[2:3])
    first_halo(2 * NT, 3 * NT)
    halo(0, 2 * NT, 3 * NT)
    _interleave(mx0)
    cp_x[2].wait()
    cp_wo.wait()
    _interleave(stage(2))
    _permute_rows(pltpu.bitcast(wo_v[...], u32), tmp, wop, 0)
    _interleave(q1[2:3])
    cp_x[3].wait()
    for c in cp_f:
        c.start()

    def step(i, carry):
        halo(i)
        q, p = qkv(i + 1), proj(i - 1)
        _interleave(q[:1] + p + q[1:], attn(i), stage(jnp.minimum(i + 2, NB - 1)), span=0.7)
        out_copy(i - 1).start()
        return carry
    lax.fori_loop(1, NB - 1, step, 0)

    bv, bi = best[0], best[1]
    rmax = jnp.max(bv, axis=0, keepdims=True)
    pos = bi + lax.broadcasted_iota(i32, (8, 128), 0).astype(f32)
    idx = jnp.min(jnp.where(bv == rmax, pos, float(S - 1))).astype(i32)
    t0 = pl.multiple_of((idx // 16) * 16, 16)
    sel = lax.broadcasted_iota(i32, (16, D), 0) == (idx - t0)
    for c in cp_f:
        c.wait()
    for i in range(NB - 2):
        out_copy(i).wait()
    res = []

    def ffn():
        xt = x_v[pl.ds(t0, 16), :].astype(f32)
        xs = jnp.sum(jnp.where(sel, xt, 0.0), axis=0, keepdims=True)
        xs16 = jnp.broadcast_to(xs, (16, D)).astype(bf16)
        gg = lax.dot_general(xs16, wg_v[...], NT_DIMS, preferred_element_type=f32)
        uu = lax.dot_general(xs16, wu_v[...], NT_DIMS, preferred_element_type=f32)
        hh = (gg * jax.nn.sigmoid(gg) * uu).astype(bf16)
        y = jnp.dot(hh, wd_v[...], preferred_element_type=f32)
        gs = jax.nn.sigmoid(jnp.sum(xs * gw, axis=-1, keepdims=True))
        res.append(y * jax.nn.sigmoid(rmax[:, 0:1]) * (1.0 - gs))

    _interleave(proj(NB - 2) + [(1, ffn)], attn(NB - 1))
    tp = pl.multiple_of(jnp.minimum(t0, (NB - 1) * M - 16), 16)
    ot = out_v[pl.ds(tp, 16), :].astype(f32)
    out_v[pl.ds(tp, 16), :] = jnp.where(lax.broadcasted_iota(i32, (16, D), 0) == idx - tp,
                                        ot + res[0], ot).astype(bf16)
    out_copy(NB - 2).start()
    tq = pl.multiple_of(jnp.minimum(t0, (NB - 2) * M - 16), 16)
    fix = pltpu.make_async_copy(out_v.at[pl.ds(tq, 16)], out_hbm.at[0, pl.ds(tq, 16)], osem.at[0])
    fix.start()
    _interleave(proj(NB - 1, (idx, res[0])))
    fix.wait()
    out_copy(NB - 2).wait()
    for p0 in range(0, M, PM):
        last_copy(p0).wait()


@jax.jit
def pallas_gated_mix__sliding_local_dilated__moe_arch_mod__prompt_kernel(
        A_x, A_wqkv, A_wo, B_x, B_w_r, B_w_gate, B_w_up, B_w_down, gate_w):
    del B_x
    hbm = pl.BlockSpec(memory_space=pl.ANY)
    vmem = pl.BlockSpec(memory_space=pltpu.VMEM)
    return pl.pallas_call(
        _kernel,
        out_shape=jax.ShapeDtypeStruct((1, S, D), bf16),
        in_specs=[hbm, hbm, hbm, vmem, hbm, hbm, hbm, vmem],
        out_specs=hbm,
        scratch_shapes=[
            pltpu.VMEM((S, D), bf16),
            pltpu.VMEM((3, D, D), bf16),
            pltpu.VMEM((D, D), bf16),
            pltpu.VMEM((F, D), bf16),
            pltpu.VMEM((F, D), bf16),
            pltpu.VMEM((F, D), bf16),
            pltpu.VMEM((NT, D // 2, 128), u32),
            pltpu.VMEM((3 * D // 2, D), u32),
            pltpu.VMEM((D // 2, D), u32),
            pltpu.VMEM((2, 3 * NT, M + HALO, 128), f32),
            pltpu.VMEM((NW, M, 128), f32),
            pltpu.VMEM((2, M // 2, D), u32),
            pltpu.VMEM((S // 2, D), u32),
            pltpu.VMEM((S, 128), f32),
            pltpu.VMEM((2, 8, 128), f32),
            pltpu.VMEM((S, D), bf16),
            pltpu.SemaphoreType.DMA((11,)),
            pltpu.SemaphoreType.DMA((NB,)),
            pltpu.SemaphoreType.DMA((M // PM,)),
        ],
        compiler_params=pltpu.CompilerParams(
            vmem_limit_bytes=100 << 20,
            flags={"XLA_TPU_EVENLY_DISTRIBUTE_CRITICAL_NODES": True},
        ),
        name="gmix",
    )(A_x, A_wqkv, A_wo, B_w_r, B_w_gate.T, B_w_up.T, B_w_down, gate_w)
```
